```python
import jax
import jax.numpy as jnp

def _softmax(x, axis=-1):
    return jax.nn.softmax(x, axis=axis)
def _gelu(x):
    return jax.nn.gelu(x, approximate=True)
def _silu(x):
    return jax.nn.silu(x)
def _sigmoid(x):
    return jax.nn.sigmoid(x)
def _layernorm(x, axis=-1, eps=1e-5):
    m = jnp.mean(x, axis=axis, keepdims=True)
    v = jnp.var(x, axis=axis, keepdims=True)
    return (x - m) / jnp.sqrt(v + eps)
def _scatter_add(tgt, idx, src, axis=0):
    return tgt.at[idx].add(src)
def _segment_sum(src, seg, n):
    return jax.ops.segment_sum(src, seg, n)
class _Rng:
    def __init__(self, key):
        self._k = key
    def _next(self):
        self._k, sub = jax.random.split(self._k)
        return sub
    def normal(self, shape):
        return jax.random.normal(self._next(), shape, dtype=jnp.bfloat16)
    def randint(self, lo, hi, shape):
        return jax.random.randint(self._next(), shape, lo, hi, dtype=jnp.int32)
    def uniform(self, shape, lo=0.0, hi=1.0):
        return jax.random.uniform(self._next(), shape, jnp.bfloat16, lo, hi)
    def permutation(self, n):
        return jax.random.permutation(self._next(), n)


kernel_name = 'concat_heads__ssm_conv_h3__compressed_kv_cla__prompt'

def setup_inputs():
    _rng = _Rng(jax.random.key(int.from_bytes(__import__("os").urandom(4), "little")))
    _w = (lambda a: (lambda t: t.astype(jnp.bfloat16) if jnp.issubdtype(t.dtype, jnp.floating) else t)(jnp.asarray(a)))
    def _A_setup():
        B, S, D = 1, 2048, 448
        ks = 4
        return {
            "q": _w((lambda *s: _rng.normal(s) * 0.05)(B, S, D)),
            "k": _w((lambda *s: _rng.normal(s) * 0.05)(B, S, D)),
            "v": _w((lambda *s: _rng.normal(s) * 0.05)(B, S, D)),
            "shift_k": _w((lambda *s: _rng.normal(s) * 0.05)(D, ks) * 0.5),
            "ssm_k": _w((lambda *s: _rng.normal(s) * 0.05)(D, S) * (1.0 / S ** 0.5)),
            "ssm_D": _w((lambda *s: _rng.normal(s) * 0.05)(D)),
        }
    _A_in = _A_setup()

    def _B_setup():
        B, H, Sq, Sk, D, M = 1, 16, 2048, 2048, 256, 448
        Dc = 4 * D
        return {
            "x": _w((lambda *s: _rng.normal(s) * 0.05)(B, Sq, M)),
            "c_kv": _w((lambda *s: _rng.normal(s) * 0.05)(B, Sk, Dc)),
            "w_q": _w((lambda *s: _rng.normal(s) * 0.05)(M, H, D) * (M ** -0.5)),
            "w_uk": _w((lambda *s: _rng.normal(s) * 0.05)(Dc, H, D) * (Dc ** -0.5)),
            "w_uv": _w((lambda *s: _rng.normal(s) * 0.05)(Dc, H, D) * (Dc ** -0.5)),
            "w_o": _w((lambda *s: _rng.normal(s) * 0.05)(H, D, M) * ((H * D) ** -0.5)),
        }
    _B_in = _B_setup()

    return {
        "A_q": _A_in["q"],
        "A_k": _A_in["k"],
        "A_v": _A_in["v"],
        "A_shift_k": _A_in["shift_k"],
        "A_ssm_k": _A_in["ssm_k"],
        "A_ssm_D": _A_in["ssm_D"],
        "B_x": _B_in["x"],
        "B_c_kv": _B_in["c_kv"],
        "B_w_q": _B_in["w_q"],
        "B_w_uk": _B_in["w_uk"],
        "B_w_uv": _B_in["w_uv"],
        "B_w_o": _B_in["w_o"],
    }

def reference(A_q, A_k, A_v, A_shift_k, A_ssm_k, A_ssm_D, B_x, B_c_kv, B_w_q, B_w_uk, B_w_uv, B_w_o):
    def _A_ref(q, k, v, shift_k, ssm_k, ssm_D):
        B, S, D = q.shape
        ks = shift_k.shape[-1]
        k_pad = jnp.pad(k, ((0, 0), (ks - 1, 0), (0, 0)))
        k_shift = jnp.zeros_like(k)
        for t in range(ks):
            k_shift = k_shift + k_pad[:, t:t + S, :] * shift_k[:, ks - 1 - t][None, None, :]
        kv = k_shift * v
        L = 2 * S
        kv_pad = jnp.pad(kv, ((0, 0), (0, S), (0, 0)))
        kf_pad = jnp.pad(ssm_k, ((0, 0), (0, S)))
        kv_f = (lambda x, axes=(-2,-1): jnp.fft.rfft2(x.astype(jnp.float32), axes=axes))(kv_pad[:, None, :, :], axes=(1, 2))
        kf_f = (lambda x, axes=(-2,-1): jnp.fft.rfft2(x.astype(jnp.float32), axes=axes))(kf_pad[:, None, :], axes=(1, 2))
        kf_f = (lambda x, *d: x.transpose(*d))(kf_f, 1, 2, 0)
        y_f = kv_f * kf_f[None, :, :, :]
        y = (lambda x, s, axes=(-2,-1): jnp.fft.irfft2(x, s=s, axes=axes).astype(jnp.bfloat16))(y_f, (1, L), axes=(1, 2))[:, 0, :S, :]
        y = y + kv * ssm_D[None, None, :]
        return q * y

    def _B_ref(x, c_kv, w_q, w_uk, w_uv, w_o):
        B, Sq, M = x.shape[0], x.shape[1], x.shape[2]
        Sk = c_kv.shape[1]
        H, D = w_q.shape[1], w_q.shape[2]
        q = jnp.einsum("bqm,mhd->bhqd", x, w_q)
        k = jnp.einsum("bkc,chd->bhkd", c_kv, w_uk)
        v = jnp.einsum("bkc,chd->bhkd", c_kv, w_uv)
        scores = jnp.einsum("bhqd,bhkd->bhqk", q, k) * (D ** -0.5)
        off = Sk - Sq
        qi = jnp.arange(Sq)[:, None]
        kj = jnp.arange(Sk)[None, :]
        cmask = kj <= (qi + off)
        scores = jnp.where(cmask[None, None], scores, -1e9)
        p = _softmax(scores, axis=-1)
        ctx = jnp.einsum("bhqk,bhkd->bhqd", p, v)
        return jnp.einsum("bhqd,hdm->bqm", ctx, w_o)

    a = _A_ref(A_q, A_k, A_v, A_shift_k, A_ssm_k, A_ssm_D)
    b = _B_ref(B_x, B_c_kv, B_w_q, B_w_uk, B_w_uv, B_w_o)
    return jnp.concatenate([a, b], axis=-1)
```

```python
import jax
import jax.numpy as jnp
import numpy as np
import jax.experimental.pallas as pl
import jax.experimental.pallas.tpu as pltpu

S = 2048
H = 16
DH = 256
M = 448
MP = 512
DC = 1024
BQ = 512
T = 128
CB = 32
NCB = M // CB
NA = S // T
QSCALE = 1.4426950408889634 / 16.0
NT = (((1,), (1,)), ((), ()))
f32 = jnp.float32
bf16 = jnp.bfloat16


def _dft():
    b = np.arange(T)[:, None].astype(np.float64)
    th = 2.0 * np.pi * (np.arange(T)[None, :] + 0.25) / T
    return np.concatenate([np.cos(th * b), np.sin(th * b)], axis=1).astype(np.float32)


def _stack(u):
    return jnp.concatenate([u[:, a * T:(a + 1) * T] for a in range(NA)], axis=0)


def conv_part(aq_ref, ak_ref, av_ref, sk_ref, w_ref, par):
    k = ak_ref[...].astype(f32)
    lane = jax.lax.broadcasted_iota(jnp.int32, (CB, S), 1)
    ks = k * par[:, 0:1]
    for j in range(1, 4):
        ks = ks + jnp.where(lane >= j, pltpu.roll(k, j, 1), 0.0) * par[:, j:j + 1]
    kv = (ks * av_ref[...].astype(f32)).astype(bf16)
    w = w_ref[...]
    U = jnp.dot(_stack(kv), w, preferred_element_type=f32)
    K = jnp.dot(_stack(sk_ref[...]), w, preferred_element_type=f32)
    ur = [U[a * CB:(a + 1) * CB, :T] for a in range(NA)]
    ui = [U[a * CB:(a + 1) * CB, T:] for a in range(NA)]
    kr0 = [K[a * CB:(a + 1) * CB, :T] for a in range(NA)]
    ki0 = [K[a * CB:(a + 1) * CB, T:] for a in range(NA)]
    kr = [kr0[0]] + [kr0[a] + ki0[a - 1] for a in range(1, NA)]
    ki = [ki0[0]] + [ki0[a] - kr0[a - 1] for a in range(1, NA)]
    zs = []
    for a in range(NA):
        zr = zi = None
        for b in range(a + 1):
            tr = ur[a - b] * kr[b] - ui[a - b] * ki[b]
            ti = ur[a - b] * ki[b] + ui[a - b] * kr[b]
            zr = tr if zr is None else zr + tr
            zi = ti if zi is None else zi + ti
        zs.append(jnp.concatenate([zr, zi], axis=1).astype(bf16))
    y = jax.lax.dot_general(jnp.concatenate(zs, axis=0), w, NT, preferred_element_type=f32)
    y = jnp.concatenate([y[a * CB:(a + 1) * CB, :] for a in range(NA)], axis=1) * (1.0 / T)
    y = y + kv.astype(f32) * par[:, 4:5]
    return (aq_ref[...].astype(f32) * y).astype(bf16)


def kern(aq_ref, ak_ref, av_ref, sk_ref, par_ref, w_ref, xt_ref, c_ref, wq_hbm, wk_hbm, wv_hbm, wo_ref,
         o_ref, x_s, q_s, kv_s, acc_s, at_s, par_s, wq_b, wk_b, wv_b, wq_s, wkv_s, wo_s, sems):
    h = pl.program_id(0)
    pair = h // 2
    slot = pair % 2

    def copies(p, sl):
        return [pltpu.make_async_copy(src.bitcast(jnp.int32).at[:, p, :], dst.at[sl], sems.at[i, sl])
                for i, (src, dst) in enumerate(((wq_hbm, wq_b), (wk_hbm, wk_b), (wv_hbm, wv_b)))]

    @pl.when(h == 0)
    def _():
        for cp in copies(0, 0):
            cp.start()
        x_s[:, M:] = jnp.zeros((S, MP - M), bf16)
        x_s[:, :M] = xt_ref[...].T
        acc_s[...] = jnp.zeros_like(acc_s)
        at_s[M:, :] = jnp.zeros((MP - M, S), bf16)
        wq_s[M:, :] = jnp.zeros((MP - M, DH), bf16)
        wo_s[:MP - M, :] = jnp.zeros((MP - M, DH), bf16)
        par_s[...] = par_ref[...].astype(f32).T

    @pl.when(h % 2 == 0)
    def _():
        for cp in copies(pair, slot):
            cp.wait()

        @pl.when(pair + 1 < H // 2)
        def _():
            for cp in copies(pair + 1, 1 - slot):
                cp.start()

    sh = (16 - 16 * (h % 2)).astype(jnp.int32)

    def unpack(buf):
        u = (buf[slot] << sh) & jnp.int32(-65536)
        return pltpu.bitcast(u, f32).astype(bf16)

    wq_s[:M, :] = unpack(wq_b)
    wkv_s[:, :DH] = unpack(wk_b)
    wkv_s[:, DH:] = unpack(wv_b)
    wo_s[MP - M:, :] = wo_ref[0]

    q_s[...] = (jnp.dot(x_s[...], wq_s[...], preferred_element_type=f32) * QSCALE).astype(bf16)
    kv_s[...] = jnp.dot(c_ref[...], wkv_s[...], preferred_element_type=f32).astype(bf16)

    c0 = pl.multiple_of(jnp.minimum(h, NCB - 1) * CB, CB)
    at_s[pl.ds(c0, CB), :] = conv_part(aq_ref, ak_ref, av_ref, sk_ref, w_ref, par_s[pl.ds(c0, CB), :])

    tri = (jax.lax.broadcasted_iota(jnp.int32, (T, T), 1) <= jax.lax.broadcasted_iota(jnp.int32, (T, T), 0))
    nsub = BQ // T
    for i in range(S // BQ):
        r0 = i * BQ
        sd = [jax.lax.dot_general(q_s[r0 + j * T:r0 + BQ, :], kv_s[r0 + j * T:r0 + (j + 1) * T, :DH], NT,
                                  preferred_element_type=f32) for j in range(nsub)]
        if i > 0:
            sf = jax.lax.dot_general(q_s[r0:r0 + BQ, :], kv_s[0:r0, :DH], NT, preferred_element_type=f32)
        ps, ls = [], []
        for ii in range(nsub):
            parts = [sf[ii * T:(ii + 1) * T, :]] if i > 0 else []
            for j in range(ii + 1):
                t = sd[j][(ii - j) * T:(ii - j + 1) * T, :]
                parts.append(jnp.where(tri, t, -1e9) if j == ii else t)
            s = jnp.concatenate(parts, axis=1) if len(parts) > 1 else parts[0]
            m = jnp.max(s, axis=-1, keepdims=True)
            p = jnp.exp2(s - m)
            ls.append(jnp.sum(p, axis=-1, keepdims=True))
            ps.append(p.astype(bf16))
        cd = [jnp.dot(jnp.concatenate([ps[ii][:, r0 + j * T:r0 + (j + 1) * T] for ii in range(j, nsub)], axis=0),
                      kv_s[r0 + j * T:r0 + (j + 1) * T, DH:], preferred_element_type=f32) for j in range(nsub)]
        if i > 0:
            cf = jnp.dot(jnp.concatenate([p_[:, :r0] for p_ in ps], axis=0), kv_s[0:r0, DH:],
                         preferred_element_type=f32)
        cs = []
        for ii in range(nsub):
            t = cf[ii * T:(ii + 1) * T, :] if i > 0 else None
            for j in range(ii + 1):
                d = cd[j][(ii - j) * T:(ii - j + 1) * T, :]
                t = d if t is None else t + d
            cs.append((t * (1.0 / ls[ii])).astype(bf16))
        ctx = jnp.concatenate(cs, axis=0)
        acc_s[r0:r0 + BQ, :] += jax.lax.dot_general(ctx, wo_s[...], NT, preferred_element_type=f32)

    @pl.when(h == H - 1)
    def _():
        o_ref[:, MP:] = acc_s[:, T:].astype(bf16)
        o_ref[:, :MP - T] = at_s[:MP - T, :].T
        lane = jax.lax.broadcasted_iota(jnp.int32, (S, T), 1)
        o_ref[:, MP - T:MP] = jnp.where(lane < M - (MP - T), at_s[MP - T:, :].T, acc_s[:, :T].astype(bf16))


@jax.jit
def pallas_concat_heads__ssm_conv_h3__compressed_kv_cla__prompt_kernel(A_q, A_k, A_v, A_shift_k, A_ssm_k, A_ssm_D, B_x, B_c_kv, B_w_q, B_w_uk, B_w_uv, B_w_o):
    tr = lambda a: jnp.swapaxes(a[0], 0, 1)
    par = jnp.concatenate([A_shift_k.T, A_ssm_D[None, :], jnp.zeros((3, M), bf16)], axis=0)
    w = jnp.asarray(_dft()).astype(bf16)
    cblk = pl.BlockSpec((CB, S), lambda h: (jnp.minimum(h, NCB - 1), 0))
    full = lambda shp: pl.BlockSpec(shp, lambda h: (0,) * len(shp))
    hbm = pl.BlockSpec(memory_space=pl.ANY)
    out = pl.pallas_call(
        kern,
        grid=(H,),
        in_specs=[cblk, cblk, cblk, cblk, full((8, M)), full((T, 2 * T)), full((M, S)), full((S, DC)),
                  hbm, hbm, hbm, pl.BlockSpec((1, M, DH), lambda h: (h, 0, 0))],
        out_specs=full((S, 2 * M)),
        out_shape=jax.ShapeDtypeStruct((S, 2 * M), bf16),
        scratch_shapes=[
            pltpu.VMEM((S, MP), bf16),
            pltpu.VMEM((S, DH), bf16),
            pltpu.VMEM((S, 2 * DH), bf16),
            pltpu.VMEM((S, MP), f32),
            pltpu.VMEM((MP, S), bf16),
            pltpu.VMEM((M, 8), f32),
            pltpu.VMEM((2, M, DH), jnp.int32),
            pltpu.VMEM((2, DC, DH), jnp.int32),
            pltpu.VMEM((2, DC, DH), jnp.int32),
            pltpu.VMEM((MP, DH), bf16),
            pltpu.VMEM((DC, 2 * DH), bf16),
            pltpu.VMEM((MP, DH), bf16),
            pltpu.SemaphoreType.DMA((3, 2)),
        ],
        compiler_params=pltpu.CompilerParams(
            dimension_semantics=("arbitrary",), vmem_limit_bytes=100 * 1024 * 1024),
    )(tr(A_q), tr(A_k), tr(A_v), A_ssm_k, par, w, tr(B_x), B_c_kv[0], B_w_q, B_w_uk, B_w_uv,
      jnp.swapaxes(B_w_o, 1, 2))
    return out[None]
```

```python
import jax
import jax.numpy as jnp
import numpy as np
import jax.experimental.pallas as pl
import jax.experimental.pallas.tpu as pltpu

S = 2048
H = 16
DH = 256
M = 448
MP = 512
DC = 1024
BQ = 512
T = 128
CB = 32
NCB = M // CB
NA = S // T
QSCALE = 1.4426950408889634 / 16.0
NT = (((1,), (1,)), ((), ()))
f32 = jnp.float32
bf16 = jnp.bfloat16


def _dft():
    b = np.arange(T)[:, None].astype(np.float64)
    th = 2.0 * np.pi * (np.arange(T)[None, :] + 0.25) / T
    return np.concatenate([np.cos(th * b), np.sin(th * b)], axis=1).astype(np.float32)


def _stack(u):
    return jnp.concatenate([u[:, a * T:(a + 1) * T] for a in range(NA)], axis=0)


def conv_part(aq_ref, ak_ref, av_ref, sk_ref, w_ref, par, at_s, c0, z_s):
    k = ak_ref[...].astype(f32)
    lane = jax.lax.broadcasted_iota(jnp.int32, (CB, S), 1)
    ks = k * par[:, 0:1]
    for j in range(1, 4):
        ks = ks + jnp.where(lane >= j, pltpu.roll(k, j, 1), 0.0) * par[:, j:j + 1]
    kv = (ks * av_ref[...].astype(f32)).astype(bf16)
    yield
    w = w_ref[...]
    U = jnp.dot(_stack(kv), w, preferred_element_type=f32)
    K = jnp.dot(_stack(sk_ref[...]), w, preferred_element_type=f32)
    ur = [U[a * CB:(a + 1) * CB, :T] for a in range(NA)]
    ui = [U[a * CB:(a + 1) * CB, T:] for a in range(NA)]
    kr0 = [K[a * CB:(a + 1) * CB, :T] for a in range(NA)]
    ki0 = [K[a * CB:(a + 1) * CB, T:] for a in range(NA)]
    kr = [kr0[0]] + [kr0[a] + ki0[a - 1] for a in range(1, NA)]
    ki = [ki0[0]] + [ki0[a] - kr0[a - 1] for a in range(1, NA)]
    yield
    zs = []
    for a in range(NA):
        zr = zi = None
        for b in range(a + 1):
            tr = ur[a - b] * kr[b] - ui[a - b] * ki[b]
            ti = ur[a - b] * ki[b] + ui[a - b] * kr[b]
            zr = tr if zr is None else zr + tr
            zi = ti if zi is None else zi + ti
        z_s[a * CB:(a + 1) * CB, :] = jnp.concatenate([zr, zi], axis=1).astype(bf16)
        if a in (5, 7, 9, 11, 12, 13, 14, 15):
            yield
    y = jax.lax.dot_general(z_s[...], w, NT, preferred_element_type=f32)
    y = jnp.concatenate([y[a * CB:(a + 1) * CB, :] for a in range(NA)], axis=1) * (1.0 / T)
    y = y + kv.astype(f32) * par[:, 4:5]
    at_s[pl.ds(c0, CB), :] = (aq_ref[...].astype(f32) * y).astype(bf16)
    yield


def kern(aq_ref, ak_ref, av_ref, sk_ref, par_ref, w_ref, xt_hbm, c_hbm, wq_hbm, wk_hbm, wv_hbm, wo_ref,
         o_ref, z_s, p_s, xt_ref, c_ref, x_s, q_s, kv_s, acc_s, at_s, par_s, wq_b, wk_b, wv_b, wq_s, wkv_s, wo_s, sems, sems2):
    h = pl.program_id(0)
    pair = h // 2
    slot = pair % 2

    def copies(p, sl):
        return [pltpu.make_async_copy(src.bitcast(jnp.int32).at[:, p, :], dst.at[sl], sems.at[i, sl])
                for i, (src, dst) in enumerate(((wq_hbm, wq_b), (wk_hbm, wk_b), (wv_hbm, wv_b)))]

    x_cp = pltpu.make_async_copy(xt_hbm, xt_ref, sems2.at[0])
    c_cp = pltpu.make_async_copy(c_hbm, c_ref, sems2.at[1])

    @pl.when(h == 0)
    def _():
        c0_ = copies(0, 0)
        for cp in (x_cp, c0_[0], c0_[1], c_cp, c0_[2]):
            cp.start()
        x_s[:, M:] = jnp.zeros((S, MP - M), bf16)
        acc_s[...] = jnp.zeros_like(acc_s)
        at_s[M:, :] = jnp.zeros((MP - M, S), bf16)
        wq_s[M:, :] = jnp.zeros((MP - M, DH), bf16)
        wo_s[:MP - M, :] = jnp.zeros((MP - M, DH), bf16)
        par_s[...] = par_ref[...].astype(f32).T
        x_cp.wait()
        x_s[:, :M] = xt_ref[...].T

    sh = (16 - 16 * (h % 2)).astype(jnp.int32)

    def unpack(buf):
        u = (buf[slot] << sh) & jnp.int32(-65536)
        return pltpu.bitcast(u, f32).astype(bf16)

    even = h % 2 == 0
    pl.when(even)(lambda: copies(pair, slot)[0].wait())
    wq_s[:M, :] = unpack(wq_b)
    wo_s[MP - M:, :] = wo_ref[0]

    c0 = pl.multiple_of(jnp.minimum(h, NCB - 1) * CB, CB)
    conv = conv_part(aq_ref, ak_ref, av_ref, sk_ref, w_ref, par_s[pl.ds(c0, CB), :], at_s, c0, z_s)
    PM = 512
    for i in range(S // PM):
        rows = slice(i * PM, (i + 1) * PM)
        next(conv, None)
        q_s[rows, :] = (jnp.dot(x_s[rows, :], wq_s[...], preferred_element_type=f32) * QSCALE).astype(bf16)
    pl.when(even)(lambda: copies(pair, slot)[1].wait())
    pl.when(h == 0)(lambda: c_cp.wait())
    for n, buf in enumerate((wk_b, wv_b)):
        cols = slice(n * DH, (n + 1) * DH)
        if n == 1:
            @pl.when(even)
            def _():
                copies(pair, slot)[2].wait()

                @pl.when(pair + 1 < H // 2)
                def _():
                    for cp in copies(pair + 1, 1 - slot):
                        cp.start()
        wkv_s[:, cols] = unpack(buf)
        for i in range(S // PM):
            rows = slice(i * PM, (i + 1) * PM)
            if n == 1:
                next(conv, None)
            kv_s[rows, cols] = jnp.dot(c_ref[rows, :], wkv_s[:, cols], preferred_element_type=f32).astype(bf16)

    tri = (jax.lax.broadcasted_iota(jnp.int32, (T, T), 1) <= jax.lax.broadcasted_iota(jnp.int32, (T, T), 0))
    nsub = BQ // T
    st = {}

    def qk(i):
        r0 = i * BQ
        sd, sf = [], []
        for j in range(nsub):
            sd.append(jax.lax.dot_general(q_s[r0 + j * T:r0 + BQ, :], kv_s[r0 + j * T:r0 + (j + 1) * T, :DH], NT,
                                          preferred_element_type=f32))
            if j % 2 == 1:
                yield
        for n in range(i):
            sf.append(jax.lax.dot_general(q_s[r0:r0 + BQ, :], kv_s[n * BQ:(n + 1) * BQ, :DH], NT,
                                          preferred_element_type=f32))
            yield
        st["s", i] = (sd, sf)

    def sm(i):
        r0 = i * BQ
        sd, sf = st.pop(("s", i))
        ps, ls = [], []
        for ii in range(nsub):
            parts = [f[ii * T:(ii + 1) * T, :] for f in sf]
            for j in range(ii + 1):
                t = sd[j][(ii - j) * T:(ii - j + 1) * T, :]
                parts.append(jnp.where(tri, t, -1e9) if j == ii else t)
            s = jnp.concatenate(parts, axis=1) if len(parts) > 1 else parts[0]
            for half in range(2):
                sh_ = s[half * 64:(half + 1) * 64]
                m = jnp.max(sh_, axis=-1, keepdims=True)
                p = jnp.exp2(sh_ - m)
                ls.append(jnp.sum(p, axis=-1, keepdims=True))
                p_s[r0 + ii * T + half * 64:r0 + ii * T + half * 64 + 64, :r0 + (ii + 1) * T] = p.astype(bf16)
                yield
        ls = [jnp.concatenate(ls[2 * ii:2 * ii + 2], axis=0) for ii in range(nsub)]
        st["p", i] = (ps, ls)

    def pv(i):
        r0 = i * BQ
        ps, ls = st.pop(("p", i))
        cd = []
        for j in range(nsub):
            cd.append(jnp.dot(p_s[r0 + j * T:r0 + BQ, r0 + j * T:r0 + (j + 1) * T],
                              kv_s[r0 + j * T:r0 + (j + 1) * T, DH:], preferred_element_type=f32))
            if j % 2 == 1:
                yield
        cf = None
        for n in range(i):
            d = jnp.dot(p_s[r0:r0 + BQ, n * BQ:(n + 1) * BQ],
                        kv_s[n * BQ:(n + 1) * BQ, DH:], preferred_element_type=f32)
            cf = d if cf is None else cf + d
            yield
        cs = []
        for ii in range(nsub):
            t = cf[ii * T:(ii + 1) * T, :] if i > 0 else None
            for j in range(ii + 1):
                d = cd[j][(ii - j) * T:(ii - j + 1) * T, :]
                t = d if t is None else t + d
            cs.append((t * (1.0 / ls[ii])).astype(bf16))
        ctx = jnp.concatenate(cs, axis=0)
        acc_s[r0:r0 + BQ, :] += jax.lax.dot_general(ctx, wo_s[...], NT, preferred_element_type=f32)
        yield

    def chain(*gs):
        for g in gs:
            yield from g

    def both(mx, nm, vp, nv):
        done = 0
        for t in range(nm):
            next(mx, None)
            want = ((t + 1) * nv + nm - 1) // nm
            while done < want:
                next(vp, None)
                done += 1
        for _ in mx:
            pass
        for _ in vp:
            pass

    for _ in qk(3):
        next(conv, None)
    both(qk(2), 4, sm(3), 8)
    both(chain(pv(3), qk(1)), 9, sm(2), 8)
    both(chain(pv(2), qk(0)), 7, sm(1), 8)
    both(pv(1), 4, sm(0), 8)
    for _ in pv(0):
        pass
    for _ in conv:
        pass

    @pl.when(h == H - 1)
    def _():
        o_ref[:, MP:] = acc_s[:, T:].astype(bf16)
        o_ref[:, :MP - T] = at_s[:MP - T, :].T
        lane = jax.lax.broadcasted_iota(jnp.int32, (S, T), 1)
        o_ref[:, MP - T:MP] = jnp.where(lane < M - (MP - T), at_s[MP - T:, :].T, acc_s[:, :T].astype(bf16))


@jax.jit
def pallas_concat_heads__ssm_conv_h3__compressed_kv_cla__prompt_kernel(A_q, A_k, A_v, A_shift_k, A_ssm_k, A_ssm_D, B_x, B_c_kv, B_w_q, B_w_uk, B_w_uv, B_w_o):
    tr = lambda a: jnp.swapaxes(a[0], 0, 1)
    par = jnp.concatenate([A_shift_k.T, A_ssm_D[None, :], jnp.zeros((3, M), bf16)], axis=0)
    w = jnp.asarray(_dft()).astype(bf16)
    cblk = pl.BlockSpec((CB, S), lambda h: (jnp.minimum(h, NCB - 1), 0))
    full = lambda shp: pl.BlockSpec(shp, lambda h: (0,) * len(shp))
    hbm = pl.BlockSpec(memory_space=pl.ANY)
    out = pl.pallas_call(
        kern,
        grid=(H,),
        in_specs=[cblk, cblk, cblk, cblk, full((8, M)), full((T, 2 * T)), hbm, hbm,
                  hbm, hbm, hbm, pl.BlockSpec((1, M, DH), lambda h: (h, 0, 0))],
        out_specs=full((S, 2 * M)),
        out_shape=jax.ShapeDtypeStruct((S, 2 * M), bf16),
        scratch_shapes=[
            pltpu.VMEM((NA * CB, 2 * T), bf16),
            pltpu.VMEM((S, S), bf16),
            pltpu.VMEM((M, S), bf16),
            pltpu.VMEM((S, DC), bf16),
            pltpu.VMEM((S, MP), bf16),
            pltpu.VMEM((S, DH), bf16),
            pltpu.VMEM((S, 2 * DH), bf16),
            pltpu.VMEM((S, MP), f32),
            pltpu.VMEM((MP, S), bf16),
            pltpu.VMEM((M, 8), f32),
            pltpu.VMEM((2, M, DH), jnp.int32),
            pltpu.VMEM((2, DC, DH), jnp.int32),
            pltpu.VMEM((2, DC, DH), jnp.int32),
            pltpu.VMEM((MP, DH), bf16),
            pltpu.VMEM((DC, 2 * DH), bf16),
            pltpu.VMEM((MP, DH), bf16),
            pltpu.SemaphoreType.DMA((3, 2)),
            pltpu.SemaphoreType.DMA((2,)),
        ],
        compiler_params=pltpu.CompilerParams(
            dimension_semantics=("arbitrary",), vmem_limit_bytes=100 * 1024 * 1024),
    )(tr(A_q), tr(A_k), tr(A_v), A_ssm_k, par, w, tr(B_x), B_c_kv[0], B_w_q, B_w_uk, B_w_uv,
      jnp.swapaxes(B_w_o, 1, 2))
    return out[None]
```
